```python
import jax
import jax.numpy as jnp

def _softmax(x, axis=-1):
    return jax.nn.softmax(x, axis=axis)
def _gelu(x):
    return jax.nn.gelu(x, approximate=True)
def _silu(x):
    return jax.nn.silu(x)
def _sigmoid(x):
    return jax.nn.sigmoid(x)
def _layernorm(x, axis=-1, eps=1e-5):
    m = jnp.mean(x, axis=axis, keepdims=True)
    v = jnp.var(x, axis=axis, keepdims=True)
    return (x - m) / jnp.sqrt(v + eps)
def _scatter_add(tgt, idx, src, axis=0):
    return tgt.at[idx].add(src)
def _segment_sum(src, seg, n):
    return jax.ops.segment_sum(src, seg, n)
class _Rng:
    def __init__(self, key):
        self._k = key
    def _next(self):
        self._k, sub = jax.random.split(self._k)
        return sub
    def normal(self, shape):
        return jax.random.normal(self._next(), shape, dtype=jnp.bfloat16)
    def randint(self, lo, hi, shape):
        return jax.random.randint(self._next(), shape, lo, hi, dtype=jnp.int32)
    def uniform(self, shape, lo=0.0, hi=1.0):
        return jax.random.uniform(self._next(), shape, jnp.bfloat16, lo, hi)
    def permutation(self, n):
        return jax.random.permutation(self._next(), n)


kernel_name = 'sequential_preLN__grouped_kv_mqa__glu_gated_swiglu__prompt'

def _fwd_setup_inputs():
    _rng = _Rng(jax.random.key(int.from_bytes(__import__("os").urandom(4), "little")))
    _w = (lambda a: (lambda t: t.astype(jnp.bfloat16) if jnp.issubdtype(t.dtype, jnp.floating) else t)(jnp.asarray(a)))
    def _A_setup():
        B, S, D, H = 1, 2048, 512, 32
        Dh = D // H
        return {
            "x": _w((lambda *s: _rng.normal(s) * 0.05)(B, S, D)),
            "wq": _w((lambda *s: _rng.normal(s) * 0.05)(D, H * Dh)),
            "wk": _w((lambda *s: _rng.normal(s) * 0.05)(D, Dh)),
            "wv": _w((lambda *s: _rng.normal(s) * 0.05)(D, Dh)),
            "wo": _w((lambda *s: _rng.normal(s) * 0.05)(H * Dh, D)),
        }
    _A_in = _A_setup()

    def _B_setup():
        B, S, D, F = 1, 2048, 512, 1376
        return {
            "x": _w((lambda *s: _rng.normal(s) * 0.05)(B, S, D)),
            "w1": _w((lambda *s: _rng.normal(s) * 0.05)(D, F) * (2.0 / D) ** 0.5),
            "w3": _w((lambda *s: _rng.normal(s) * 0.05)(D, F) * (2.0 / D) ** 0.5),
            "w2": _w((lambda *s: _rng.normal(s) * 0.05)(F, D) * (2.0 / F) ** 0.5),
        }
    _B_in = _B_setup()

    return {
        "A_x": _A_in["x"],
        "A_wq": _A_in["wq"],
        "A_wk": _A_in["wk"],
        "A_wv": _A_in["wv"],
        "A_wo": _A_in["wo"],
        "B_x": _B_in["x"],
        "B_w1": _B_in["w1"],
        "B_w3": _B_in["w3"],
        "B_w2": _B_in["w2"],
    }

def _fwd_reference(A_x, A_wq, A_wk, A_wv, A_wo, B_x, B_w1, B_w3, B_w2):
    def _A_ref(x, wq, wk, wv, wo):
        B, S, D = x.shape
        H = 32
        Dh = D // H
        q = (lambda x, *d: x.transpose(*d))((x @ wq).reshape(B, S, H, Dh), 0, 2, 1, 3)
        k = x @ wk
        v = x @ wv
        scores = jnp.einsum("bhqd,bkd->bhqk", q, k) * (Dh ** -0.5)
        p = _softmax(scores, axis=-1)
        o = jnp.einsum("bhqk,bkd->bhqd", p, v)
        return (lambda x, *d: x.transpose(*d))(o, 0, 2, 1, 3).reshape(B, S, H * Dh) @ wo

    def _B_ref(x, w1, w3, w2):
        gate = jnp.einsum("bsd,df->bsf", x, w1)
        up = jnp.einsum("bsd,df->bsf", x, w3)
        h = _silu(gate) * up
        out = jnp.einsum("bsf,fd->bsd", h, w2)
        return out

    x = A_x
    h = x + _A_ref(_layernorm(x, axis=-1), A_wq, A_wk, A_wv, A_wo)
    h2 = h + _B_ref(_layernorm(h, axis=-1), B_w1, B_w3, B_w2)
    return h2


def setup_inputs():
    _inp = _fwd_setup_inputs()
    _gk = jax.random.fold_in(jax.random.key(int.from_bytes(__import__("os").urandom(4), "little")), 2**31 - 1)
    _shapes = [[1, 2048, 512]]
    _dtypes = ['bfloat16']
    _gks = jax.random.split(_gk, len(_shapes))
    _gs = [jax.random.normal(k, s, dtype=jnp.dtype(d)) * 0.05 for k, s, d in zip(_gks, _shapes, _dtypes)]
    _inp["grad_out"] = _gs[0]
    return _inp

def reference(A_x, A_wq, A_wk, A_wv, A_wo, B_w1, B_w3, B_w2, B_x, grad_out):
    _const = dict(B_x=B_x)
    def _f(*_d):
        return _fwd_reference(**{'A_x': _d[0], 'A_wq': _d[1], 'A_wk': _d[2], 'A_wv': _d[3], 'A_wo': _d[4], 'B_w1': _d[5], 'B_w3': _d[6], 'B_w2': _d[7], **_const})
    _out, _vjp = jax.vjp(_f, A_x, A_wq, A_wk, A_wv, A_wo, B_w1, B_w3, B_w2)
    _grads = _vjp(grad_out)
    _out0 = jnp.asarray(_out)
    return (_out0, *[jnp.asarray(_g) for _g in _grads])
```

```python
import jax
import jax.numpy as jnp
from jax import lax
import jax.experimental.pallas as pl
import jax.experimental.pallas.tpu as pltpu

f32 = jnp.float32
bf16 = jnp.bfloat16
u32 = jnp.uint32

S, D, H, DH, F = 2048, 512, 32, 16, 1376
TQ = 128
NQ = S // TQ
W = 512
HG = W // TQ
G = H // HG
CK = 128
CB = 128
EPS = 1e-5
LOG2E = 1.4426950408889634
LN2 = 0.6931471805599453

NN = (((1,), (0,)), ((), ()))
NT = (((1,), (1,)), ((), ()))
TN = (((0,), (0,)), ((), ()))
TT = (((0,), (1,)), ((), ()))


def _dot(a, b, dn=NN):
    return lax.dot_general(a, b, dn, preferred_element_type=f32)


def _rows(g, n):
    if isinstance(g, int):
        return pl.ds(g * n, n)
    return pl.ds(pl.multiple_of(g * n, n), n)


def _ln_stats(hT):
    mu = jnp.mean(hT, axis=0, keepdims=True)
    xc = hT - mu
    var = jnp.mean(xc * xc, axis=0, keepdims=True)
    rstd = lax.rsqrt(var + EPS)
    return xc * rstd, rstd


def _ln_bwd(dy, xhat, rstd):
    m1 = jnp.mean(dy, axis=0, keepdims=True)
    m2 = jnp.mean(dy * xhat, axis=0, keepdims=True)
    return rstd * (dy - m1 - xhat * m2)


def _cat(xT, g):
    return jnp.concatenate(
        [xT[(g * HG + j) * DH:(g * HG + j + 1) * DH, :] for j in range(HG)], axis=1)


def _kernel(x_ref, wq_ref, wkT_ref, wvT_ref, wo_ref, w1T, w3T, w2_ref, g_ref,
            h2_ref, dx_ref, dwq_ref, dwkT_ref, dwvT_ref, dwo_ref, dw1T_ref, dw3T_ref, dw2_ref,
            wqT, woT, w1n, w3n, w2T, xT, ln1T, st1, kvT, kn, vn, qcat,
            sbuf, pbuf, mbuf, ocat, docat, dlcat, dqcat, dkvT, dxp,
            awq, awo, aw1, aw3, aw2):
    i = pl.program_id(0)

    def s_pass(q, c):
        sl = pl.ds(c * CK, CK)
        s = _dot(kn[sl, :], q)
        sbuf[sl, :] = s
        return jnp.max(s.reshape(CK // 8, 8, W), axis=0)

    @pl.when(i == 0)
    def _phase0():
        wqT[...] = wq_ref[...].T
        woT[...] = wo_ref[...].T
        w1n[...] = w1T[...].T
        w3n[...] = w3T[...].T
        w2T[...] = w2_ref[...].T
        awq[...] = jnp.zeros_like(awq)
        awo[...] = jnp.zeros_like(awo)
        aw1[...] = jnp.zeros_like(aw1)
        aw3[...] = jnp.zeros_like(aw3)
        aw2[...] = jnp.zeros_like(aw2)
        dkvT[...] = jnp.zeros_like(dkvT)
        RB = 256
        for b in range(S // RB):
            cs = pl.ds(b * RB, RB)
            xb = x_ref[cs, :].T
            xT[:, cs] = xb
            xh, rstd = _ln_stats(xb.astype(f32))
            st1[:, cs] = rstd
            lb = xh.astype(bf16)
            ln1T[:, cs] = lb
            qT = _dot(wqT[...], lb) * (0.25 * LOG2E)
            qTb = qT.astype(bf16)
            for t in range(RB // TQ):
                blk = b * (RB // TQ) + t
                qblk = qTb[:, t * TQ:(t + 1) * TQ]
                for g in range(G):
                    qcat[pl.ds((blk * G + g) * DH, DH), :] = _cat(qblk, g)
            kT = _dot(wkT_ref[...], lb)
            vT = _dot(wvT_ref[...], lb)
            kvT[0:DH, cs] = kT.astype(bf16)
            kvT[DH:2 * DH, cs] = vT.astype(bf16)
            kn[cs, :] = _dot(lb, wkT_ref[...], TT).astype(bf16)
            vn[cs, :] = _dot(lb, wvT_ref[...], TT).astype(bf16)
        q0 = qcat[0:DH, :]
        mx = None
        for c in range(S // CK):
            t = s_pass(q0, c)
            mx = t if mx is None else jnp.maximum(mx, t)
        mbuf[...] = jnp.broadcast_to(jnp.max(mx, axis=0, keepdims=True), (8, W))

    def fwd_body(g, m):
        nxt = jnp.minimum(i * G + g + 1, NQ * G - 1)
        q = qcat[_rows(nxt, DH), :]
        mx = None
        ls = None
        oacc = None
        for c in range(S // CK):
            sl = pl.ds(c * CK, CK)
            p = jnp.exp2(sbuf[sl, :].reshape(CK // 8, 8, W) - m[None])
            ps = jnp.sum(p, axis=0)
            ls = ps if ls is None else ls + ps
            pb = p.reshape(CK, W).astype(bf16)
            pbuf[pl.ds(pl.multiple_of(g * (S // 2) + c * (CK // 2), CK // 2), CK // 2), :] = (
                pltpu.bitcast(pb, u32))
            t = s_pass(q, c)
            mx = t if mx is None else jnp.maximum(mx, t)
            o = _dot(kvT[DH:2 * DH, sl], pb)
            oacc = o if oacc is None else oacc + o
        l = jnp.sum(ls, axis=0, keepdims=True)
        rl = 1.0 / l
        ocat[_rows(g, DH), :] = oacc * rl
        dlcat[pl.ds(g, 1), :] = rl
        return jnp.broadcast_to(jnp.max(mx, axis=0, keepdims=True), (8, W))

    mbuf[...] = lax.fori_loop(0, G, fwd_body, mbuf[...])

    cs = pl.ds(pl.multiple_of(i * TQ, TQ), TQ)
    oT = jnp.concatenate(
        [ocat[g * DH:(g + 1) * DH, j * TQ:(j + 1) * TQ] for g in range(G) for j in range(HG)],
        axis=0)
    oTb = oT.astype(bf16)
    hT = xT[:, cs].astype(f32) + _dot(woT[...], oTb)
    xh2, rstd2 = _ln_stats(hT)
    ln2b = xh2.astype(bf16)
    gate = _dot(w1T[...], ln2b)
    up = _dot(w3T[...], ln2b)
    sig = jax.nn.sigmoid(gate)
    silu = gate * sig
    hhb = (silu * up).astype(bf16)
    h2T = hT + _dot(w2T[...], hhb)
    h2_ref[...] = h2T.astype(bf16).T

    gTb = g_ref[...].T
    dhh = _dot(w2_ref[...], gTb)
    dupb = (dhh * silu).astype(bf16)
    dgateb = (dhh * up * (sig * (1.0 + gate * (1.0 - sig)))).astype(bf16)
    aw2[...] += _dot(hhb, gTb, NT)
    aw1[...] += _dot(dgateb, ln2b, NT)
    aw3[...] += _dot(dupb, ln2b, NT)
    dln2 = _dot(w1n[...], dgateb) + _dot(w3n[...], dupb)
    dhT = gTb.astype(f32) + _ln_bwd(dln2, xh2, rstd2)
    dhTb = dhT.astype(bf16)
    doT = _dot(wo_ref[...], dhTb)
    awo[...] += _dot(oTb, dhTb, NT)
    for g in range(G):
        rl = dlcat[g:g + 1, :]
        dos = _cat(doT, g) * rl
        docat[g * DH:(g + 1) * DH, :] = dos.astype(bf16)
        dlcat[g:g + 1, :] = jnp.sum(dos * ocat[g * DH:(g + 1) * DH, :], axis=0, keepdims=True)

    def bwd_body(g, carry):
        do = docat[_rows(g, DH), :]
        q = qcat[_rows(i * G + g, DH), :]
        dl = dlcat[pl.ds(g, 1), :]
        n = S // CB

        def dp(c):
            return _dot(vn[pl.ds(c * CB, CB), :], do)

        def rest(c, dpv, dq):
            sl = pl.ds(c * CB, CB)
            pb = pltpu.bitcast(
                pbuf[pl.ds(pl.multiple_of(g * (S // 2) + c * (CB // 2), CB // 2), CB // 2), :], bf16)
            ds = (pb.astype(f32) * (dpv - dl)).astype(bf16)
            dkvT[DH:2 * DH, sl] += _dot(do, pb, NT)
            dkvT[0:DH, sl] += _dot(q, ds, NT)
            t = _dot(kvT[0:DH, sl], ds)
            return t if dq is None else dq + t

        dq = None
        cur = dp(0)
        for c in range(n):
            nx = dp(c + 1) if c + 1 < n else None
            dq = rest(c, cur, dq)
            cur = nx
        dqcat[_rows(g, DH), :] = dq
        return carry

    lax.fori_loop(0, G, bwd_body, 0)

    dqT = jnp.concatenate(
        [dqcat[g * DH:(g + 1) * DH, j * TQ:(j + 1) * TQ] for g in range(G) for j in range(HG)],
        axis=0)
    dqTb = (dqT * 0.25).astype(bf16)
    l1b = ln1T[:, cs]
    awq[...] += _dot(l1b, dqTb, NT)
    dln1 = _dot(wq_ref[...], dqTb)
    x1 = xT[:, cs].astype(f32)
    rstd1 = st1[:, cs]
    xh1 = (x1 - jnp.mean(x1, axis=0, keepdims=True)) * rstd1
    dxp[:, cs] = dhT + _ln_bwd(dln1, xh1, rstd1)

    @pl.when(i == NQ - 1)
    def _final():
        dwq_ref[...] = awq[...].astype(bf16)
        dwo_ref[...] = awo[...].astype(bf16)
        dw1T_ref[...] = aw1[...].astype(bf16)
        dw3T_ref[...] = aw3[...].astype(bf16)
        dw2_ref[...] = aw2[...].astype(bf16)
        dkb = (dkvT[0:DH, :] * LN2).astype(bf16)
        dvb = dkvT[DH:2 * DH, :].astype(bf16)
        l1 = ln1T[...]
        dwkT_ref[...] = _dot(dkb, l1, NT).astype(bf16)
        dwvT_ref[...] = _dot(dvb, l1, NT).astype(bf16)
        RB = 256
        for b in range(S // RB):
            bs = pl.ds(b * RB, RB)
            dl1 = (_dot(wkT_ref[...], dkb[:, b * RB:(b + 1) * RB], TN)
                   + _dot(wvT_ref[...], dvb[:, b * RB:(b + 1) * RB], TN))
            xb = xT[:, bs].astype(f32)
            r1 = st1[:, bs]
            xh = (xb - jnp.mean(xb, axis=0, keepdims=True)) * r1
            dxT = dxp[:, bs] + _ln_bwd(dl1, xh, r1)
            dx_ref[bs, :] = dxT.astype(bf16).T


@jax.jit
def pallas_sequential_preLN__grouped_kv_mqa__glu_gated_swiglu__prompt_kernel(
    A_x: jax.Array,
    A_wq: jax.Array,
    A_wk: jax.Array,
    A_wv: jax.Array,
    A_wo: jax.Array,
    B_x: jax.Array,
    B_w1: jax.Array,
    B_w3: jax.Array,
    B_w2: jax.Array,
    grad_out: jax.Array,
):
    del B_x
    x = A_x.reshape(S, D)
    g = grad_out.reshape(S, D)

    def whole(shape):
        return pl.BlockSpec(shape, lambda i: (0,) * len(shape))

    blk = pl.BlockSpec((TQ, D), lambda i: (i, 0))
    vm = pltpu.VMEM
    out_shape = (
        jax.ShapeDtypeStruct((S, D), bf16),
        jax.ShapeDtypeStruct((S, D), bf16),
        jax.ShapeDtypeStruct((D, D), bf16),
        jax.ShapeDtypeStruct((DH, D), bf16),
        jax.ShapeDtypeStruct((DH, D), bf16),
        jax.ShapeDtypeStruct((D, D), bf16),
        jax.ShapeDtypeStruct((F, D), bf16),
        jax.ShapeDtypeStruct((F, D), bf16),
        jax.ShapeDtypeStruct((F, D), bf16),
    )
    outs = pl.pallas_call(
        _kernel,
        grid=(NQ,),
        in_specs=[whole((S, D)), whole((D, D)), whole((DH, D)), whole((DH, D)), whole((D, D)),
                  whole((F, D)), whole((F, D)), whole((F, D)), blk],
        out_specs=[blk, whole((S, D)), whole((D, D)), whole((DH, D)), whole((DH, D)),
                   whole((D, D)), whole((F, D)), whole((F, D)), whole((F, D))],
        out_shape=out_shape,
        scratch_shapes=[
            vm((D, D), bf16), vm((D, D), bf16), vm((D, F), bf16), vm((D, F), bf16), vm((D, F), bf16),
            vm((D, S), bf16), vm((D, S), bf16), vm((1, S), f32),
            vm((2 * DH, S), bf16), vm((S, DH), bf16), vm((S, DH), bf16),
            vm((NQ * G * DH, W), bf16),
            vm((S, W), f32), vm((G * S // 2, W), u32), vm((8, W), f32),
            vm((G * DH, W), f32), vm((G * DH, W), bf16), vm((G, W), f32), vm((G * DH, W), f32),
            vm((2 * DH, S), f32), vm((D, S), f32),
            vm((D, D), f32), vm((D, D), f32), vm((F, D), f32), vm((F, D), f32), vm((F, D), f32),
        ],
        compiler_params=pltpu.CompilerParams(
            dimension_semantics=("arbitrary",),
            vmem_limit_bytes=110 * 1024 * 1024,
        ),
    )(x, A_wq, A_wk.T, A_wv.T, A_wo, B_w1.T, B_w3.T, B_w2, g)
    h2, dx, dwq, dwkT, dwvT, dwo, dw1T, dw3T, dw2 = outs
    return (h2.reshape(1, S, D), dx.reshape(1, S, D), dwq, dwkT.T, dwvT.T, dwo, dw1T.T, dw3T.T, dw2)
```

```python
import jax
import jax.numpy as jnp
from jax import lax
import jax.experimental.pallas as pl
import jax.experimental.pallas.tpu as pltpu

f32 = jnp.float32
bf16 = jnp.bfloat16
u32 = jnp.uint32

S, D, H, DH, F = 2048, 512, 32, 16, 1376
TQ = 256
NQ = S // TQ
W = 512
HG = W // TQ
G = H // HG
CK = 128
CB = 128
FU = 2
BP = 2
FS = F // 2
RB = 256
EPS = 1e-5
LOG2E = 1.4426950408889634
LN2 = 0.6931471805599453

NN = (((1,), (0,)), ((), ()))
NT = (((1,), (1,)), ((), ()))


def _dot(a, b, dn=NN):
    return lax.dot_general(a, b, dn, preferred_element_type=f32)


def _rows(g, n):
    if isinstance(g, int):
        return pl.ds(g * n, n)
    return pl.ds(pl.multiple_of(g * n, n), n)


def _ln_stats(hT):
    mu = jnp.mean(hT, axis=0, keepdims=True)
    xc = hT - mu
    var = jnp.mean(xc * xc, axis=0, keepdims=True)
    rstd = lax.rsqrt(var + EPS)
    return xc * rstd, rstd


def _ln_bwd(dy, xhat, rstd):
    m1 = jnp.mean(dy, axis=0, keepdims=True)
    m2 = jnp.mean(dy * xhat, axis=0, keepdims=True)
    return rstd * (dy - m1 - xhat * m2)


def _cat(xT, g):
    if HG == 1:
        return xT[g * DH:(g + 1) * DH, :]
    return jnp.concatenate(
        [xT[(g * HG + j) * DH:(g * HG + j + 1) * DH, :] for j in range(HG)], axis=1)


def _uncat(ref):
    return jnp.concatenate(
        [ref[g * DH:(g + 1) * DH, j * TQ:(j + 1) * TQ] for g in range(G) for j in range(HG)],
        axis=0)


def _kernel(x_hbm, wq_hbm, wkT_hbm, wvT_hbm, wo_hbm, w1T_hbm, w3T_hbm, w2_hbm, g_hbm,
            h2_ref, dx_hbm, dwq_hbm, dwkT_hbm, dwvT_hbm, dwo_hbm, dw1T_hbm, dw3T_hbm, dw2_hbm,
            xs, gs, wq, wqkvT, wo, woT, w1T, w1n, w3T, w3n, w2, w2T,
            xT, gT, ln1T, st1, kvT, kn, vn, qcat,
            sbuf, sbuf2, pbuf, mbuf, lbuf, dpbuf, ocat, docat, dlcat, dqcat, dkvT, dhs, dl1s, dkvo,
            awq, awo, aw1, aw3, aw2, isem, osem):
    i = pl.program_id(0)

    def in_copy(k):
        src, dst = [
            (x_hbm, xs), (wq_hbm, wq), (wkT_hbm, wqkvT.at[pl.ds(D, DH)]),
            (wvT_hbm, wqkvT.at[pl.ds(D + DH, DH)]), (wo_hbm, wo), (w2_hbm, w2),
            (w1T_hbm, w1T), (w3T_hbm, w3T), (g_hbm, gs)][k]
        return pltpu.make_async_copy(src, dst, isem.at[k])

    def out_copy(k, b=0):
        if k == 0:
            return pltpu.make_async_copy(xs.at[pl.ds(b * RB, RB)], dx_hbm.at[pl.ds(b * RB, RB)],
                                         osem.at[8 + b])
        src, dst = [None, (wq, dwq_hbm), (dkvo.at[pl.ds(0, DH)], dwkT_hbm),
                    (dkvo.at[pl.ds(DH, DH)], dwvT_hbm), (wo, dwo_hbm), (w1T, dw1T_hbm),
                    (w3T, dw3T_hbm), (w2, dw2_hbm)][k]
        return pltpu.make_async_copy(src, dst, osem.at[k])

    sbs = (sbuf, sbuf2)

    def s_pass(q, c, sb):
        sl = pl.ds(c * CK, CK)
        s = _dot(kn[sl, :], q)
        sb[sl, :] = s
        return jnp.max(s.reshape(CK // 8, 8, W), axis=0)

    @pl.when(i == 0)
    def _phase0():
        for k in (1, 2, 3, 0):
            in_copy(k).start()
        awq[...] = jnp.zeros_like(awq)
        awo[...] = jnp.zeros_like(awo)
        aw1[...] = jnp.zeros_like(aw1)
        aw3[...] = jnp.zeros_like(aw3)
        aw2[...] = jnp.zeros_like(aw2)
        dkvT[...] = jnp.zeros_like(dkvT)
        in_copy(2).wait()
        in_copy(3).wait()
        in_copy(1).wait()
        wqkvT[0:D, :] = wq[...].T
        in_copy(0).wait()
        for k in range(4, 9):
            in_copy(k).start()
        for b in range(S // RB):
            cs = pl.ds(b * RB, RB)
            xb = xs[cs, :].T
            xT[:, cs] = xb
            xh, rstd = _ln_stats(xb.astype(f32))
            st1[0:1, cs] = jnp.mean(xb.astype(f32), axis=0, keepdims=True)
            st1[1:2, cs] = rstd
            lb = xh.astype(bf16)
            ln1T[:, cs] = lb
            qkv = _dot(wqkvT[...], lb)
            qTb = (qkv[0:D] * (0.25 * LOG2E)).astype(bf16)
            for t in range(RB // TQ):
                blk = b * (RB // TQ) + t
                qblk = qTb[:, t * TQ:(t + 1) * TQ]
                for g in range(G):
                    qcat[pl.ds((blk * G + g) * DH, DH), :] = _cat(qblk, g)
            kv = qkv[D:D + 2 * DH]
            kvT[:, cs] = kv.astype(bf16)
            kvn = jnp.concatenate([kv, jnp.zeros((128 - 2 * DH, RB), f32)], axis=0).T
            kn[cs, :] = kvn[:, 0:DH].astype(bf16)
            vn[cs, :] = kvn[:, DH:2 * DH].astype(bf16)
        for k in range(4, 9):
            in_copy(k).wait()
        gT[...] = gs[0:TQ, :].T
        woT[...] = wo[...].T
        w2T[...] = w2[...].T
        w1n[...] = w1T[...].T
        w3n[...] = w3T[...].T
        for u in range(FU):
            q0 = qcat[u * DH:(u + 1) * DH, :]
            mx = None
            for c in range(S // CK):
                t = s_pass(q0, c, sbs[u])
                mx = t if mx is None else jnp.maximum(mx, t)
            mbuf[u * 8:(u + 1) * 8, :] = mx

    def fwd_group(g, m, sb, more):
        m = jnp.broadcast_to(jnp.max(m, axis=0, keepdims=True), (8, W))
        if more:
            q = qcat[_rows(i * G + g + FU, DH), :]
        mx = None
        ls = None
        oacc = None
        for c in range(S // CK):
            sl = pl.ds(c * CK, CK)
            p = jnp.exp2(sb[sl, :].reshape(CK // 8, 8, W) - m[None])
            pb = p.reshape(CK, W).astype(bf16)
            t2 = p.reshape(CK // 32, 2, 2, 8, W)
            ps = jnp.sum((t2[:, 0, 0] + t2[:, 0, 1]) + (t2[:, 1, 0] + t2[:, 1, 1]), axis=0)
            ls = ps if ls is None else ls + ps
            pbuf[pl.ds(pl.multiple_of(g * (S // 2) + c * (CK // 2), CK // 2), CK // 2), :] = (
                pltpu.bitcast(pb, u32))
            if more:
                t = s_pass(q, c, sb)
                mx = t if mx is None else jnp.maximum(mx, t)
            o = _dot(kvT[DH:2 * DH, sl], pb)
            oacc = o if oacc is None else oacc + o
        ocat[_rows(g, DH), :] = oacc
        lbuf[_rows(g, 8), :] = ls
        if more:
            return mx

    def fwd_body(t, ms):
        return tuple(fwd_group(t * FU + u, ms[u], sbs[u], True) for u in range(FU))

    last = i == NQ - 1
    ms = lax.fori_loop(0, G // FU - last.astype(jnp.int32), fwd_body,
                       tuple(mbuf[u * 8:(u + 1) * 8, :] for u in range(FU)))
    for u in range(FU):
        mbuf[u * 8:(u + 1) * 8, :] = ms[u]

    @pl.when(last)
    def _last_groups():
        for u in range(FU):
            fwd_group(G - FU + u, mbuf[u * 8:(u + 1) * 8, :], sbs[u], False)

    cs = pl.ds(pl.multiple_of(i * TQ, TQ), TQ)
    gTb = gT[...]
    dhh_a = _dot(w2[0:FS, :], gTb)
    rls = []
    for g in range(G):
        rl = 1.0 / jnp.sum(lbuf[g * 8:(g + 1) * 8, :], axis=0, keepdims=True)
        rls.append(rl)
        ocat[g * DH:(g + 1) * DH, :] = ocat[g * DH:(g + 1) * DH, :] * rl
    oTb = _uncat(ocat).astype(bf16)
    hT = xT[:, cs].astype(f32) + _dot(woT[...], oTb)
    dhh = jnp.concatenate([dhh_a, _dot(w2[FS:F, :], gTb)], axis=0)
    xh2, rstd2 = _ln_stats(hT)
    ln2b = xh2.astype(bf16)
    gate = _dot(w1T[...], ln2b)
    up = _dot(w3T[...], ln2b)
    sig = jax.nn.sigmoid(gate)
    silu = gate * sig
    hhb = (silu * up).astype(bf16)
    h2T = hT + _dot(w2T[...], hhb)
    h2_ref[...] = h2T.astype(bf16).T

    dupb = (dhh * silu).astype(bf16)
    dgateb = (dhh * up * (sig * (1.0 + gate * (1.0 - sig)))).astype(bf16)
    dln2 = _dot(w1n[...], dgateb) + _dot(w3n[...], dupb)
    aw2[...] += _dot(hhb, gTb, NT)
    aw1[...] += _dot(dgateb, ln2b, NT)
    aw3[...] += _dot(dupb, ln2b, NT)
    dhT = gTb.astype(f32) + _ln_bwd(dln2, xh2, rstd2)
    dhs[:, cs] = dhT
    dhTb = dhT.astype(bf16)
    doT = _dot(wo[...], dhTb)
    awo[...] += _dot(oTb, dhTb, NT)
    for g in range(G):
        dos = _cat(doT, g) * rls[g]
        docat[g * DH:(g + 1) * DH, :] = dos.astype(bf16)
        dlcat[pl.ds(g, 1), :] = jnp.sum(dos * ocat[g * DH:(g + 1) * DH, :], axis=0, keepdims=True)

    do0 = docat[0:DH, :]
    for c in range(BP):
        dpbuf[pl.ds(c * CB, CB), :] = _dot(vn[pl.ds(c * CB, CB), :], do0)

    @pl.when(i == NQ - 1)
    def _flush_ffn_grads():
        wo[...] = awo[...].astype(bf16)
        out_copy(4).start()
        w1T[...] = aw1[...].astype(bf16)
        out_copy(5).start()
        w3T[...] = aw3[...].astype(bf16)
        out_copy(6).start()
        w2[...] = aw2[...].astype(bf16)
        out_copy(7).start()

    def bwd_body(g, carry):
        do = docat[_rows(g, DH), :]
        q = qcat[_rows(i * G + g, DH), :]
        dl = dlcat[pl.ds(g, 1), :]
        don = docat[_rows(jnp.minimum(g + 1, G - 1), DH), :]
        n = S // CB

        def dp(c):
            if c >= n:
                dpbuf[pl.ds((c - n) * CB, CB), :] = _dot(vn[pl.ds((c - n) * CB, CB), :], don)
                return None
            if c < BP:
                return dpbuf[pl.ds(c * CB, CB), :]
            return _dot(vn[pl.ds(c * CB, CB), :], do)

        dq = None
        pend = [dp(c) for c in range(BP)]
        for c in range(n):
            sl = pl.ds(c * CB, CB)
            pb = pltpu.bitcast(
                pbuf[pl.ds(pl.multiple_of(g * (S // 2) + c * (CB // 2), CB // 2), CB // 2), :], bf16)
            ds = (pb.astype(f32) * (pend.pop(0) - dl)).astype(bf16)
            t = _dot(kvT[0:DH, sl], ds)
            dq = t if dq is None else dq + t
            pend.append(dp(c + BP))
            dkvT[0:DH, sl] += _dot(q, ds, NT)
            dkvT[DH:2 * DH, sl] += _dot(do, pb, NT)
        dqcat[_rows(g, DH), :] = dq
        return carry

    lax.fori_loop(0, G, bwd_body, 0)

    dqTb = (_uncat(dqcat) * 0.25).astype(bf16)
    dl1s[:, cs] = _dot(wq[...], dqTb)
    awq[...] += _dot(ln1T[:, cs], dqTb, NT)
    nb = jnp.minimum(i + 1, NQ - 1)
    gT[...] = gs[pl.ds(pl.multiple_of(nb * TQ, TQ), TQ), :].T

    @pl.when(i == NQ - 1)
    def _final():
        wq[...] = awq[...].astype(bf16)
        out_copy(1).start()
        scale = jnp.where(lax.broadcasted_iota(jnp.int32, (2 * DH, 1), 0) < DH, LN2, 1.0)
        dkvb = (dkvT[...] * scale).astype(bf16)
        wkv = jnp.concatenate(
            [wqkvT[D:D + 2 * DH, :].astype(f32), jnp.zeros((128 - 2 * DH, D), f32)],
            axis=0).T[:, 0:2 * DH].astype(bf16)
        T = 128
        for cb in range(S // T):
            ts = pl.ds(cb * T, T)
            dkl = _dot(wkv, dkvb[:, cb * T:(cb + 1) * T])
            s1 = s2 = None
            for r in range(D // T):
                rs = pl.ds(r * T, T)
                d = dl1s[rs, ts] + dkl[r * T:(r + 1) * T]
                dl1s[rs, ts] = d
                a1 = jnp.sum(d.reshape(T // 8, 8, T), axis=0)
                a2 = jnp.sum((d * xT[rs, ts].astype(f32)).reshape(T // 8, 8, T), axis=0)
                s1 = a1 if s1 is None else s1 + a1
                s2 = a2 if s2 is None else s2 + a2
            mu, r1 = st1[0:1, ts], st1[1:2, ts]
            m1 = jnp.sum(s1, axis=0, keepdims=True) * (1.0 / D)
            m2 = (jnp.sum(s2, axis=0, keepdims=True) * (1.0 / D) - mu * m1) * r1
            cx = r1 * r1 * m2
            c0 = cx * mu - r1 * m1
            for r in range(D // T):
                rs = pl.ds(r * T, T)
                o = dhs[rs, ts] + (r1 * dl1s[rs, ts] - cx * xT[rs, ts].astype(f32) + c0)
                xs[ts, rs] = o.astype(bf16).T
            if (cb + 1) % (RB // T) == 0:
                out_copy(0, cb // (RB // T)).start()
        dkvo[...] = _dot(dkvb, ln1T[...], NT).astype(bf16)
        out_copy(2).start()
        out_copy(3).start()
        for k in range(1, 8):
            out_copy(k).wait()
        for b in range(S // RB):
            out_copy(0, b).wait()


@jax.jit
def pallas_sequential_preLN__grouped_kv_mqa__glu_gated_swiglu__prompt_kernel(
    A_x: jax.Array,
    A_wq: jax.Array,
    A_wk: jax.Array,
    A_wv: jax.Array,
    A_wo: jax.Array,
    B_x: jax.Array,
    B_w1: jax.Array,
    B_w3: jax.Array,
    B_w2: jax.Array,
    grad_out: jax.Array,
):
    del B_x
    x = A_x.reshape(S, D)
    g = grad_out.reshape(S, D)

    hbm = pl.BlockSpec(memory_space=pl.ANY)
    blk = pl.BlockSpec((TQ, D), lambda i: (i, 0))
    vm = pltpu.VMEM
    out_shape = (
        jax.ShapeDtypeStruct((S, D), bf16),
        jax.ShapeDtypeStruct((S, D), bf16),
        jax.ShapeDtypeStruct((D, D), bf16),
        jax.ShapeDtypeStruct((DH, D), bf16),
        jax.ShapeDtypeStruct((DH, D), bf16),
        jax.ShapeDtypeStruct((D, D), bf16),
        jax.ShapeDtypeStruct((F, D), bf16),
        jax.ShapeDtypeStruct((F, D), bf16),
        jax.ShapeDtypeStruct((F, D), bf16),
    )
    outs = pl.pallas_call(
        _kernel,
        grid=(NQ,),
        in_specs=[hbm] * 9,
        out_specs=[blk] + [hbm] * 8,
        out_shape=out_shape,
        scratch_shapes=[
            vm((S, D), bf16), vm((S, D), bf16), vm((D, D), bf16), vm((D + 2 * DH, D), bf16),
            vm((D, D), bf16), vm((D, D), bf16),
            vm((F, D), bf16), vm((D, F), bf16), vm((F, D), bf16), vm((D, F), bf16),
            vm((F, D), bf16), vm((D, F), bf16),
            vm((D, S), bf16), vm((D, TQ), bf16), vm((D, S), bf16), vm((2, S), f32),
            vm((2 * DH, S), bf16), vm((S, DH), bf16), vm((S, DH), bf16),
            vm((NQ * G * DH, W), bf16),
            vm((S, W), f32), vm((S, W), f32), vm((G * S // 2, W), u32), vm((8 * FU, W), f32), vm((G * 8, W), f32),
            vm((BP * CB, W), f32),
            vm((G * DH, W), f32), vm((G * DH, W), bf16), vm((G, W), f32), vm((G * DH, W), f32),
            vm((2 * DH, S), f32), vm((D, S), f32), vm((D, S), f32), vm((2 * DH, D), bf16),
            vm((D, D), f32), vm((D, D), f32), vm((F, D), f32), vm((F, D), f32), vm((F, D), f32),
            pltpu.SemaphoreType.DMA((9,)), pltpu.SemaphoreType.DMA((8 + S // RB,)),
        ],
        compiler_params=pltpu.CompilerParams(
            dimension_semantics=("arbitrary",),
            vmem_limit_bytes=110 * 1024 * 1024,
        ),
    )(x, A_wq, A_wk.T, A_wv.T, A_wo, B_w1.T, B_w3.T, B_w2, g)
    h2, dx, dwq, dwkT, dwvT, dwo, dw1T, dw3T, dw2 = outs
    return (h2.reshape(1, S, D), dx.reshape(1, S, D), dwq, dwkT.T, dwvT.T, dwo, dw1T.T, dw3T.T, dw2)
```
